```python
import os as _os
_os.environ.setdefault("JAX_PLATFORMS", "cpu")
import jax
import jax.numpy as jnp

def _softmax(x, axis=-1):
    return jax.nn.softmax(x, axis=axis)
def _gelu(x):
    return jax.nn.gelu(x, approximate=True)
def _silu(x):
    return jax.nn.silu(x)
def _sigmoid(x):
    return jax.nn.sigmoid(x)
def _layernorm(x, axis=-1, eps=1e-5):
    m = jnp.mean(x, axis=axis, keepdims=True)
    v = jnp.var(x, axis=axis, keepdims=True)
    return (x - m) / jnp.sqrt(v + eps)
def _scatter_add(tgt, idx, src, axis=0):
    return tgt.at[idx].add(src)
def _segment_sum(src, seg, n):
    return jax.ops.segment_sum(src, seg, n)
class _Rng:
    def __init__(self, key):
        self._k = key
    def _next(self):
        self._k, sub = jax.random.split(self._k)
        return sub
    def normal(self, shape):
        return jax.random.normal(self._next(), shape, dtype=jnp.bfloat16)
    def randint(self, lo, hi, shape):
        return jax.random.randint(self._next(), shape, lo, hi, dtype=jnp.int32)
    def uniform(self, shape, lo=0.0, hi=1.0):
        return jax.random.uniform(self._next(), shape, jnp.bfloat16, lo, hi)
    def permutation(self, n):
        return jax.random.permutation(self._next(), n)


kernel_name = 'gated_mix__grouped_kv_mqa__ssm_conv_s5__prompt'

def setup_inputs():
    _rng = _Rng(jax.random.key(int.from_bytes(__import__("os").urandom(4), "little")))
    _w = (lambda a: (lambda t: t.astype(jnp.bfloat16) if jnp.issubdtype(t.dtype, jnp.floating) else t)(jnp.asarray(a)))
    def _A_setup():
        B, S, D, H = 1, 2048, 512, 32
        Dh = D // H
        return {
            "x": _w((lambda *s: _rng.normal(s) * 0.05)(B, S, D)),
            "wq": _w((lambda *s: _rng.normal(s) * 1.6)(D, H * Dh)),
            "wk": _w((lambda *s: _rng.normal(s) * 1.6)(D, Dh)),
            "wv": _w((lambda *s: _rng.normal(s) * 0.05)(D, Dh)),
            "wo": _w((lambda *s: _rng.normal(s) * 0.05)(H * Dh, D)),
        }
    _A_in = _A_setup()

    def _B_setup():
        B, S, D = 1, 2048, 512
        P = D
        Lambda_re = -0.5 * jnp.exp((lambda *s: _rng.normal(s) * 0.4)(P))
        Lambda_im = (lambda *s: _rng.normal(s) * 0.4)(P) * 1.0
        B_re = (lambda *s: _rng.normal(s) * 0.4)(P, D) * (D ** -0.5)
        B_im = (lambda *s: _rng.normal(s) * 0.4)(P, D) * (D ** -0.5)
        C_re = (lambda *s: _rng.normal(s) * 0.4)(D, P) * (P ** -0.5)
        C_im = (lambda *s: _rng.normal(s) * 0.4)(D, P) * (P ** -0.5)
        log_dt = (lambda *s: _rng.normal(s) * 0.4)(P) * 0.3 - 2.0
        Dskip = (lambda *s: _rng.normal(s) * 0.4)(D)
        return {
            "x": _w((lambda *s: _rng.normal(s) * 0.05)(B, S, D)),
            "Lambda_re": _w(Lambda_re),
            "Lambda_im": _w(Lambda_im),
            "B_re": _w(B_re),
            "B_im": _w(B_im),
            "C_re": _w(C_re),
            "C_im": _w(C_im),
            "log_dt": _w(log_dt),
            "Dskip": _w(Dskip),
        }
    _B_in = _B_setup()

    return {
        "A_x": _A_in["x"],
        "A_wq": _A_in["wq"],
        "A_wk": _A_in["wk"],
        "A_wv": _A_in["wv"],
        "A_wo": _A_in["wo"],
        "B_x": _B_in["x"],
        "B_Lambda_re": _B_in["Lambda_re"],
        "B_Lambda_im": _B_in["Lambda_im"],
        "B_B_re": _B_in["B_re"],
        "B_B_im": _B_in["B_im"],
        "B_C_re": _B_in["C_re"],
        "B_C_im": _B_in["C_im"],
        "B_log_dt": _B_in["log_dt"],
        "B_Dskip": _B_in["Dskip"],
        "gate_w": _w((lambda *s: _rng.normal(s) * 0.05)(512) * 16.0),
    }

def reference(A_x, A_wq, A_wk, A_wv, A_wo, B_x, B_Lambda_re, B_Lambda_im, B_B_re, B_B_im, B_C_re, B_C_im, B_log_dt, B_Dskip, gate_w):
    def _A_ref(x, wq, wk, wv, wo):
        B, S, D = x.shape
        H = 32
        Dh = D // H
        q = (lambda x, *d: x.transpose(*d))((x @ wq).reshape(B, S, H, Dh), 0, 2, 1, 3)
        k = x @ wk
        v = x @ wv
        scores = jnp.einsum("bhqd,bkd->bhqk", q, k) * (Dh ** -0.5)
        p = _softmax(scores, axis=-1)
        o = jnp.einsum("bhqk,bkd->bhqd", p, v)
        return (lambda x, *d: x.transpose(*d))(o, 0, 2, 1, 3).reshape(B, S, H * Dh) @ wo

    def _B_ref(x, Lambda_re, Lambda_im, B_re, B_im, C_re, C_im, log_dt, Dskip):
        Bsz, L, H = x.shape
        Lam = Lambda_re + 1j * Lambda_im
        Bmat = B_re + 1j * B_im
        Cmat = C_re + 1j * C_im
        dt = jnp.exp(log_dt)
        Lam_bar = jnp.exp(dt * Lam)
        B_bar = ((Lam_bar - 1.0) / Lam)[:, None] * Bmat
        Bu = jnp.einsum("bld,pd->blp", x + 0j, B_bar)
        h = jnp.zeros_like(Bu[:, 0, :])
        hs = []
        for t in range(L):
            h = Lam_bar[None, :] * h + Bu[:, t, :]
            hs.append(h)
        hseq = jnp.stack(hs, 1)
        y = 2.0 * jnp.einsum("blp,dp->bld", hseq, Cmat).real + x * Dskip[None, None, :]
        return y

    x = A_x
    g = _sigmoid((x * gate_w).sum(-1, keepdims=True))
    a = _A_ref(x, A_wq, A_wk, A_wv, A_wo)
    b = _B_ref(x, B_Lambda_re, B_Lambda_im, B_B_re, B_B_im, B_C_re, B_C_im, B_log_dt, B_Dskip)
    return g * a + (1 - g) * b
```

```python
import functools

import jax
import jax.numpy as jnp
from jax import lax
import jax.experimental.pallas as pl
import jax.experimental.pallas.tpu as pltpu

F32 = jnp.float32
BF16 = jnp.bfloat16

S_LEN = 2048
D = 512
H = 32
DH = 16
P = 512
TQ = 512
KC = 256
SB = 64


def _cmul(ar, ai, br, bi):
    return ar * br - ai * bi, ar * bi + ai * br


def _kernel(x_ref, wq_ref, wk_ref, wv_ref, wo_ref,
            lre_ref, lim_ref, bre_ref, bim_ref, cre_ref, cim_ref,
            ldt_ref, dskip_ref, gw_ref,
            o_ref,
            k_s, vt_s, qt_s, at_s, tab_s, car_s, sa_s, sb_s, ma_s, mb_s):
    i = pl.program_id(0)

    @pl.when(i == 0)
    def _init():
        x = x_ref[...]
        k_s[...] = jnp.dot(x, wk_ref[...], preferred_element_type=F32).astype(BF16)
        vt = lax.dot_general(wv_ref[...], x, (((0,), (1,)), ((), ())),
                             preferred_element_type=F32)
        row = lax.broadcasted_iota(jnp.int32, (DH, S_LEN), 0)
        vt_s[0:DH, :] = vt.astype(BF16)
        vt_s[DH:2 * DH, :] = jnp.where(row == 0, 1.0, 0.0).astype(BF16)

        lre = lre_ref[...].astype(F32).reshape(1, P)
        lim = lim_ref[...].astype(F32).reshape(1, P)
        dt = jnp.exp(ldt_ref[...].astype(F32).reshape(1, P)).astype(BF16).astype(F32)
        zr = dt * lre
        zi = dt * lim
        er = jnp.exp(zr)
        l1r = er * jnp.cos(zi)
        l1i = er * jnp.sin(zi)
        nr = l1r - 1.0
        ni = l1i
        den = lre * lre + lim * lim
        c_r = (nr * lre + ni * lim) / den
        c_i = (ni * lre - nr * lim) / den

        pows = [(l1r, l1i)]
        for _ in range(7):
            pr, pi = pows[-1]
            pows.append(_cmul(pr, pi, l1r, l1i))
        l8r, l8i = pows[7]
        l16r, l16i = _cmul(l8r, l8i, l8r, l8i)
        l32r, l32i = _cmul(l16r, l16i, l16r, l16i)

        rows = lax.broadcasted_iota(jnp.int32, (8, P), 0)

        def masked(vr, k):
            return jnp.where(rows >= k, jnp.broadcast_to(vr, (8, P)), 0.0)

        tab_s[0] = masked(pows[0][0], 1)
        tab_s[1] = masked(pows[0][1], 1)
        tab_s[2] = masked(pows[1][0], 2)
        tab_s[3] = masked(pows[1][1], 2)
        tab_s[4] = masked(pows[3][0], 4)
        tab_s[5] = masked(pows[3][1], 4)
        tab_s[6] = masked(l8r, 1)
        tab_s[7] = masked(l8i, 1)
        tab_s[8] = masked(l16r, 2)
        tab_s[9] = masked(l16i, 2)
        tab_s[10] = masked(l32r, 4)
        tab_s[11] = masked(l32i, 4)
        tr = jnp.zeros((8, P), F32)
        ti = jnp.zeros((8, P), F32)
        for r in range(8):
            tr = jnp.where(rows == r, jnp.broadcast_to(pows[r][0], (8, P)), tr)
            ti = jnp.where(rows == r, jnp.broadcast_to(pows[r][1], (8, P)), ti)
        tab_s[12] = tr
        tab_s[13] = ti
        tab_s[14] = jnp.broadcast_to(c_r, (8, P))
        tab_s[15] = jnp.broadcast_to(c_i, (8, P))
        car_s[...] = jnp.zeros_like(car_s)

    row0 = pl.multiple_of(i * TQ, TQ)
    xb = x_ref[pl.ds(row0, TQ), :]
    qt = lax.dot_general(wq_ref[...], xb, (((0,), (1,)), ((), ())),
                         preferred_element_type=F32)
    qt_s[...] = (qt.astype(BF16).astype(F32) * 0.25).astype(BF16)

    def qk_only(h, s_buf, m_buf):
        off = pl.multiple_of(h * DH, DH)
        qh = qt_s[pl.ds(off, DH), :]
        macc = None
        for c in range(S_LEN // KC):
            sc = jnp.dot(k_s[c * KC:(c + 1) * KC, :], qh, preferred_element_type=F32)
            s_buf[c * KC:(c + 1) * KC, :] = sc
            mc = jnp.max(sc.reshape(KC // 8, 8, TQ), axis=0)
            macc = mc if macc is None else jnp.maximum(macc, mc)
        m_buf[...] = macc

    def stage(h, s_cur, m_cur, s_nxt, m_nxt, do_qk):
        if do_qk:
            offn = pl.multiple_of((h + 1) * DH, DH)
            qh = qt_s[pl.ds(offn, DH), :]
        m = jnp.max(m_cur[...], axis=0, keepdims=True)
        macc = None
        oacc = None
        for c in range(S_LEN // KC):
            rows = slice(c * KC, (c + 1) * KC)
            if do_qk:
                sc = jnp.dot(k_s[rows, :], qh, preferred_element_type=F32)
                s_nxt[rows, :] = sc
                mc = jnp.max(sc.reshape(KC // 8, 8, TQ), axis=0)
                macc = mc if macc is None else jnp.maximum(macc, mc)
            p = jnp.exp(s_cur[rows, :] - m).astype(BF16)
            oc = jnp.dot(vt_s[:, rows], p, preferred_element_type=F32)
            oacc = oc if oacc is None else oacc + oc
        if do_qk:
            m_nxt[...] = macc
        off = pl.multiple_of(h * DH, DH)
        at_s[pl.ds(off, DH), :] = (oacc[0:DH] / oacc[DH:DH + 1]).astype(BF16)

    qk_only(0, sa_s, ma_s)

    def step(h, carry):
        lax.cond(h % 2 == 0,
                 lambda: stage(h, sa_s, ma_s, sb_s, mb_s, True),
                 lambda: stage(h, sb_s, mb_s, sa_s, ma_s, True))
        return carry

    lax.fori_loop(0, H - 1, step, 0)
    stage(H - 1, sb_s, mb_s, sa_s, ma_s, False)
    a = lax.dot_general(at_s[...], wo_ref[...], (((0,), (0,)), ((), ())),
                        preferred_element_type=F32)
    a_bf = a.astype(BF16)

    u_r = lax.dot_general(xb, bre_ref[...], (((1,), (1,)), ((), ())),
                          preferred_element_type=F32)
    u_i = lax.dot_general(xb, bim_ref[...], (((1,), (1,)), ((), ())),
                          preferred_element_type=F32)
    c_r = tab_s[14][0:1, :]
    c_i = tab_s[15][0:1, :]
    bu_r = c_r * u_r - c_i * u_i
    bu_i = c_r * u_i + c_i * u_r

    rows8 = lax.broadcasted_iota(jnp.int32, (8, P), 0)
    car_r = car_s[0:1, :]
    car_i = car_s[1:2, :]
    hs_r = []
    hs_i = []
    for sb in range(TQ // SB):
        xr = bu_r[sb * SB:(sb + 1) * SB, :].reshape(SB // 8, 8, P)
        xi = bu_i[sb * SB:(sb + 1) * SB, :].reshape(SB // 8, 8, P)
        for lvl, k in enumerate((1, 2, 4)):
            mr = tab_s[2 * lvl][None]
            mi = tab_s[2 * lvl + 1][None]
            sr = pltpu.roll(xr, k, 1)
            si = pltpu.roll(xi, k, 1)
            xr, xi = xr + mr * sr - mi * si, xi + mr * si + mi * sr
        e_r = xr[:, 7, :]
        e_i = xi[:, 7, :]
        hr = jnp.where(rows8 == 0, jnp.broadcast_to(car_r, (8, P)), pltpu.roll(e_r, 1, 0))
        hi = jnp.where(rows8 == 0, jnp.broadcast_to(car_i, (8, P)), pltpu.roll(e_i, 1, 0))
        for lvl, k in enumerate((1, 2, 4)):
            mr = tab_s[6 + 2 * lvl]
            mi = tab_s[6 + 2 * lvl + 1]
            sr = pltpu.roll(hr, k, 0)
            si = pltpu.roll(hi, k, 0)
            hr, hi = hr + mr * sr - mi * si, hi + mr * si + mi * sr
        tr = tab_s[12][None]
        ti = tab_s[13][None]
        hpr = hr[:, None, :]
        hpi = hi[:, None, :]
        fr = xr + tr * hpr - ti * hpi
        fi = xi + tr * hpi + ti * hpr
        car_r = fr[SB // 8 - 1, 7:8, :]
        car_i = fi[SB // 8 - 1, 7:8, :]
        hs_r.append(fr.reshape(SB, P))
        hs_i.append(fi.reshape(SB, P))
    car_s[0:1, :] = car_r
    car_s[1:2, :] = car_i
    h_r = jnp.concatenate(hs_r, axis=0).astype(BF16)
    h_i = jnp.concatenate(hs_i, axis=0).astype(BF16)
    yr = lax.dot_general(h_r, cre_ref[...], (((1,), (1,)), ((), ())),
                         preferred_element_type=F32)
    yi = lax.dot_general(h_i, cim_ref[...], (((1,), (1,)), ((), ())),
                         preferred_element_type=F32)
    xb32 = xb.astype(F32)
    dskip = dskip_ref[...].astype(F32).reshape(1, D)
    b = 2.0 * (yr - yi) + (xb32 * dskip).astype(BF16).astype(F32)

    gw = gw_ref[...].astype(F32).reshape(1, D)
    prod = (xb32 * gw).astype(BF16).astype(F32)
    logit = jnp.sum(prod, axis=-1, keepdims=True).astype(BF16).astype(F32)
    g = jax.nn.sigmoid(logit).astype(BF16)
    one_m_g = (1.0 - g.astype(F32)).astype(BF16).astype(F32)
    ga = (g.astype(F32) * a_bf.astype(F32)).astype(BF16).astype(F32)
    o_ref[...] = ga + one_m_g * b


@jax.jit
def pallas_gated_mix__grouped_kv_mqa__ssm_conv_s5__prompt_kernel(
    A_x, A_wq, A_wk, A_wv, A_wo, B_x, B_Lambda_re, B_Lambda_im, B_B_re, B_B_im,
    B_C_re, B_C_im, B_log_dt, B_Dskip, gate_w,
):
    x = A_x.reshape(S_LEN, D)
    full = lambda shp: pl.BlockSpec(shp, lambda i: (0,) * len(shp))
    out = pl.pallas_call(
        _kernel,
        grid=(S_LEN // TQ,),
        in_specs=[
            full((S_LEN, D)),
            full((D, H * DH)),
            full((D, DH)),
            full((D, DH)),
            full((H * DH, D)),
            full((P,)), full((P,)),
            full((P, D)), full((P, D)),
            full((D, P)), full((D, P)),
            full((P,)), full((D,)), full((D,)),
        ],
        out_specs=pl.BlockSpec((TQ, D), lambda i: (i, 0)),
        out_shape=jax.ShapeDtypeStruct((S_LEN, D), F32),
        scratch_shapes=[
            pltpu.VMEM((S_LEN, DH), BF16),
            pltpu.VMEM((2 * DH, S_LEN), BF16),
            pltpu.VMEM((D, TQ), BF16),
            pltpu.VMEM((D, TQ), BF16),
            pltpu.VMEM((16, 8, P), F32),
            pltpu.VMEM((8, P), F32),
            pltpu.VMEM((S_LEN, TQ), F32),
            pltpu.VMEM((S_LEN, TQ), F32),
            pltpu.VMEM((8, TQ), F32),
            pltpu.VMEM((8, TQ), F32),
        ],
        compiler_params=pltpu.CompilerParams(
            dimension_semantics=("arbitrary",),
            vmem_limit_bytes=100 * 1024 * 1024,
        ),
    )(x, A_wq, A_wk, A_wv, A_wo, B_Lambda_re, B_Lambda_im, B_B_re, B_B_im,
      B_C_re, B_C_im, B_log_dt, B_Dskip, gate_w)
    return out.reshape(1, S_LEN, D)
```

```python
import functools

import jax
import jax.numpy as jnp
from jax import lax
import jax.experimental.pallas as pl
import jax.experimental.pallas.tpu as pltpu

F32 = jnp.float32
BF16 = jnp.bfloat16

S_LEN = 2048
D = 512
H = 32
DH = 16
P = 512
TQ = 512
NB = S_LEN // TQ
KC = 128
NC = S_LEN // KC
RC = 128
NT = TQ // RC


def _cmul(ar, ai, br, bi):
    return ar * br - ai * bi, ar * bi + ai * br


def _kernel(x_hbm, wq_hbm, wkt_hbm, wvt_hbm, wo_hbm,
            lre_ref, lim_ref, bre_hbm, bim_hbm, cre_hbm, cim_hbm,
            ldt_ref, dskip_ref, gw_ref,
            o_ref,
            k_s, vt_s, qt_s, at_s, tab_s, car_s, s0_s, s1_s, s2_s, s3_s, m0_s, m1_s, m2_s, m3_s,
            x_ref, wq_ref, wkt_ref, wvt_ref, wo_ref, bre_ref, bim_ref, cre_ref, cim_ref, sems):
    i = pl.program_id(0)

    def x_copy(b):
        return pltpu.make_async_copy(x_hbm.at[pl.ds(b * TQ, TQ)], x_ref.at[pl.ds(b * TQ, TQ)],
                                     sems.at[b])

    w_pairs = ((wq_hbm, wq_ref), (wkt_hbm, wkt_ref), (wvt_hbm, wvt_ref), (wo_hbm, wo_ref),
               (bre_hbm, bre_ref), (bim_hbm, bim_ref), (cre_hbm, cre_ref), (cim_hbm, cim_ref))

    def w_copy(n):
        return pltpu.make_async_copy(w_pairs[n][0], w_pairs[n][1], sems.at[NB + n])

    def qk_chunk(c, qh):
        rows = slice(c * KC, (c + 1) * KC)
        return jnp.dot(k_s[rows, :], qh, preferred_element_type=F32)

    def q_slice(h, blk):
        ro = pl.multiple_of(h * DH, DH)
        co = pl.multiple_of(blk * TQ, TQ)
        return qt_s[pl.ds(ro, DH), pl.ds(co, TQ)]

    @pl.when(i == 0)
    def _init():
        x_copy(0).start()
        for n in (0, 1, 2):
            w_copy(n).start()
        for b in range(1, NB):
            x_copy(b).start()
        for n in range(3, 8):
            w_copy(n).start()

        w_copy(0).wait()
        for b in range(NB):
            x_copy(b).wait()
            qt = lax.dot_general(wq_ref[...], x_ref[b * TQ:(b + 1) * TQ, :],
                                 (((0,), (1,)), ((), ())), preferred_element_type=F32)
            qt_s[:, b * TQ:(b + 1) * TQ] = (qt.astype(BF16).astype(F32) * 0.25).astype(BF16)
        w_copy(1).wait()
        w_copy(2).wait()
        x = x_ref[...]
        k_s[...] = lax.dot_general(x, wkt_ref[...], (((1,), (1,)), ((), ())),
                                   preferred_element_type=F32).astype(BF16)
        vt = lax.dot_general(wvt_ref[...], x, (((1,), (1,)), ((), ())),
                             preferred_element_type=F32)
        row = lax.broadcasted_iota(jnp.int32, (DH, S_LEN), 0)
        vt_s[0:DH, :] = vt.astype(BF16)
        vt_s[DH:2 * DH, :] = jnp.where(row == 0, 1.0, 0.0).astype(BF16)

        lre = lre_ref[...].astype(F32).reshape(1, P)
        lim = lim_ref[...].astype(F32).reshape(1, P)
        dt = jnp.exp(ldt_ref[...].astype(F32).reshape(1, P)).astype(BF16).astype(F32)
        zr = dt * lre
        zi = dt * lim
        er = jnp.exp(zr)
        l1r = er * jnp.cos(zi)
        l1i = er * jnp.sin(zi)
        nr = l1r - 1.0
        ni = l1i
        den = lre * lre + lim * lim
        c_r = (nr * lre + ni * lim) / den
        c_i = (ni * lre - nr * lim) / den
        pows = [(l1r, l1i)]
        for _ in range(7):
            pr, pi = pows[-1]
            pows.append(_cmul(pr, pi, l1r, l1i))

        rows = lax.broadcasted_iota(jnp.int32, (8, P), 0)

        def masked(vr, k):
            return jnp.where(rows >= k, jnp.broadcast_to(vr, (8, P)), 0.0)

        tab_s[0] = masked(pows[0][0], 1)
        tab_s[1] = masked(pows[0][1], 1)
        tab_s[2] = masked(pows[1][0], 2)
        tab_s[3] = masked(pows[1][1], 2)
        tab_s[4] = masked(pows[3][0], 4)
        tab_s[5] = masked(pows[3][1], 4)
        tr = jnp.zeros((8, P), F32)
        ti = jnp.zeros((8, P), F32)
        for r in range(8):
            tr = jnp.where(rows == r, jnp.broadcast_to(pows[r][0], (8, P)), tr)
            ti = jnp.where(rows == r, jnp.broadcast_to(pows[r][1], (8, P)), ti)
        tab_s[6] = tr
        tab_s[7] = ti
        tab_s[8] = jnp.broadcast_to(c_r, (8, P))
        tab_s[9] = jnp.broadcast_to(c_i, (8, P))
        tab_s[10] = jnp.broadcast_to(pows[7][0], (8, P))
        tab_s[11] = jnp.broadcast_to(pows[7][1], (8, P))
        car_s[...] = jnp.zeros_like(car_s)

        for hh, (sbuf, mbuf) in enumerate(((s0_s, m0_s), (s1_s, m1_s))):
            qh = q_slice(hh, 0)
            macc = None
            for c in range(NC):
                sc = qk_chunk(c, qh)
                sbuf[c * KC:(c + 1) * KC, :] = sc
                mc = jnp.max(sc.reshape(KC // 8, 8, TQ), axis=0)
                macc = mc if macc is None else jnp.maximum(macc, mc)
            mbuf[...] = macc

    row0 = pl.multiple_of(i * TQ, TQ)

    def stage(h, s_cur, m_cur, s_nxt, m_nxt):
        hn = h + 2
        wrap = hn // H
        hn = hn - wrap * H
        bn = jnp.minimum(i + wrap, NB - 1)
        qh = q_slice(hn, bn)
        m = jnp.max(m_cur[...], axis=0, keepdims=True)
        macc = None
        oacc = None
        for c in range(NC):
            rows = slice(c * KC, (c + 1) * KC)
            sc = qk_chunk(c, qh)
            s_nxt[rows, :] = sc
            mc = jnp.max(sc.reshape(KC // 8, 8, TQ), axis=0)
            macc = mc if macc is None else jnp.maximum(macc, mc)
            p = jnp.exp(s_cur[rows, :] - m).astype(BF16)
            oc = jnp.dot(vt_s[:, rows], p, preferred_element_type=F32)
            oacc = oc if oacc is None else oacc + oc
        m_nxt[...] = macc
        off = pl.multiple_of(h * DH, DH)
        at_s[pl.ds(off, DH), :] = (oacc[0:DH] / oacc[DH:DH + 1]).astype(BF16)

    def step(j, carry):
        def even():
            stage(2 * j, s0_s, m0_s, s2_s, m2_s)
            stage(2 * j + 1, s1_s, m1_s, s3_s, m3_s)

        def odd():
            stage(2 * j, s2_s, m2_s, s0_s, m0_s)
            stage(2 * j + 1, s3_s, m3_s, s1_s, m1_s)

        lax.cond(j % 2 == 0, even, odd)
        return carry

    lax.fori_loop(0, H // 2, step, 0)

    def bproj(t):
        xt = x_ref[pl.ds(row0 + t * RC, RC), :]
        ur = lax.dot_general(xt, bre_ref[...], (((1,), (1,)), ((), ())),
                             preferred_element_type=F32)
        ui = lax.dot_general(xt, bim_ref[...], (((1,), (1,)), ((), ())),
                             preferred_element_type=F32)
        return ur, ui

    def scan(ur, ui):
        c_r = tab_s[8][0:1, :]
        c_i = tab_s[9][0:1, :]
        br = c_r * ur - c_i * ui
        bi = c_r * ui + c_i * ur
        G = RC // 8
        xr = br.reshape(G, 8, P)
        xi = bi.reshape(G, 8, P)
        for lvl, k in enumerate((1, 2, 4)):
            mr = tab_s[2 * lvl][None]
            mi = tab_s[2 * lvl + 1][None]
            sr = pltpu.roll(xr, k, 1)
            si = pltpu.roll(xi, k, 1)
            xr, xi = xr + mr * sr - mi * si, xi + mr * si + mi * sr
        hr = car_s[0:1, :]
        hi = car_s[1:2, :]
        tr = tab_s[6]
        ti = tab_s[7]
        outs_r = []
        outs_i = []
        for g in range(G):
            hb_r = jnp.broadcast_to(hr, (8, P))
            hb_i = jnp.broadcast_to(hi, (8, P))
            fr = xr[g] + tr * hb_r - ti * hb_i
            fi = xi[g] + tr * hb_i + ti * hb_r
            outs_r.append(fr)
            outs_i.append(fi)
            hr = fr[7:8, :]
            hi = fi[7:8, :]
        car_s[0:1, :] = hr
        car_s[1:2, :] = hi
        return (jnp.concatenate(outs_r, axis=0).astype(BF16),
                jnp.concatenate(outs_i, axis=0).astype(BF16))

    def finish(t, h_r, h_i):
        cols = slice(t * RC, (t + 1) * RC)
        a = lax.dot_general(at_s[:, cols], wo_ref[...], (((0,), (0,)), ((), ())),
                            preferred_element_type=F32)
        a_bf = a.astype(BF16)
        yr = lax.dot_general(h_r, cre_ref[...], (((1,), (1,)), ((), ())),
                             preferred_element_type=F32)
        yi = lax.dot_general(h_i, cim_ref[...], (((1,), (1,)), ((), ())),
                             preferred_element_type=F32)
        xt32 = x_ref[pl.ds(row0 + t * RC, RC), :].astype(F32)
        dskip = dskip_ref[...].astype(F32).reshape(1, D)
        b = 2.0 * (yr - yi) + (xt32 * dskip).astype(BF16).astype(F32)
        gw = gw_ref[...].astype(F32).reshape(1, D)
        prod = (xt32 * gw).astype(BF16).astype(F32)
        logit = jnp.sum(prod, axis=-1, keepdims=True).astype(BF16).astype(F32)
        g = jax.nn.sigmoid(logit).astype(BF16)
        one_m_g = (1.0 - g.astype(F32)).astype(BF16).astype(F32)
        ga = (g.astype(F32) * a_bf.astype(F32)).astype(BF16).astype(F32)
        o_ref[cols, :] = ga + one_m_g * b

    @pl.when(i == 0)
    def _wait_rest():
        for n in range(3, 8):
            w_copy(n).wait()

    u = bproj(0)
    for t in range(NT):
        u_next = bproj(t + 1) if t + 1 < NT else None
        h_r, h_i = scan(*u)
        finish(t, h_r, h_i)
        u = u_next


@jax.jit
def pallas_gated_mix__grouped_kv_mqa__ssm_conv_s5__prompt_kernel(
    A_x, A_wq, A_wk, A_wv, A_wo, B_x, B_Lambda_re, B_Lambda_im, B_B_re, B_B_im,
    B_C_re, B_C_im, B_log_dt, B_Dskip, gate_w,
):
    x = A_x.reshape(S_LEN, D)
    full = lambda shp: pl.BlockSpec(shp, lambda i: (0,) * len(shp))
    hbm = pl.BlockSpec(memory_space=pl.ANY)
    out = pl.pallas_call(
        _kernel,
        grid=(NB,),
        in_specs=[
            hbm, hbm, hbm, hbm, hbm,
            full((P,)), full((P,)),
            hbm, hbm, hbm, hbm,
            full((P,)), full((D,)), full((D,)),
        ],
        out_specs=pl.BlockSpec((TQ, D), lambda i: (i, 0)),
        out_shape=jax.ShapeDtypeStruct((S_LEN, D), F32),
        scratch_shapes=[
            pltpu.VMEM((S_LEN, DH), BF16),
            pltpu.VMEM((2 * DH, S_LEN), BF16),
            pltpu.VMEM((D, S_LEN), BF16),
            pltpu.VMEM((D, TQ), BF16),
            pltpu.VMEM((12, 8, P), F32),
            pltpu.VMEM((8, P), F32),
            pltpu.VMEM((S_LEN, TQ), F32),
            pltpu.VMEM((S_LEN, TQ), F32),
            pltpu.VMEM((S_LEN, TQ), F32),
            pltpu.VMEM((S_LEN, TQ), F32),
            pltpu.VMEM((8, TQ), F32),
            pltpu.VMEM((8, TQ), F32),
            pltpu.VMEM((8, TQ), F32),
            pltpu.VMEM((8, TQ), F32),
            pltpu.VMEM((S_LEN, D), BF16),
            pltpu.VMEM((D, H * DH), BF16),
            pltpu.VMEM((DH, D), BF16),
            pltpu.VMEM((DH, D), BF16),
            pltpu.VMEM((H * DH, D), BF16),
            pltpu.VMEM((P, D), BF16),
            pltpu.VMEM((P, D), BF16),
            pltpu.VMEM((D, P), BF16),
            pltpu.VMEM((D, P), BF16),
            pltpu.SemaphoreType.DMA((NB + 8,)),
        ],
        compiler_params=pltpu.CompilerParams(
            dimension_semantics=("arbitrary",),
            vmem_limit_bytes=100 * 1024 * 1024,
        ),
    )(x, A_wq, A_wk.T, A_wv.T, A_wo, B_Lambda_re, B_Lambda_im, B_B_re, B_B_im,
      B_C_re, B_C_im, B_log_dt, B_Dskip, gate_w)
    return out.reshape(1, S_LEN, D)
```

```python
import jax
import jax.numpy as jnp
from jax import lax
import jax.experimental.pallas as pl
import jax.experimental.pallas.tpu as pltpu

F32 = jnp.float32
BF16 = jnp.bfloat16

S_LEN = 2048
D = 512
H = 32
DH = 16
P = 512
TQ = 512
NB = S_LEN // TQ
KC = 128
NC = S_LEN // KC
HB = 4
RC = 128
NT = TQ // RC
N_W = 8


def _cmul(ar, ai, br, bi):
    return ar * br - ai * bi, ar * bi + ai * br


def _kernel(x_hbm, wq_hbm, wkt_hbm, wvt_hbm, wo_hbm,
            lre_ref, lim_ref, bre_hbm, bim_hbm, cre_hbm, cim_hbm,
            ldt_ref, dskip_ref, gw_ref,
            o_hbm,
            k_s, vt_s, qt_s, at_s, tab_s, car_s,
            x_ref, wq_ref, wkt_ref, wvt_ref, wo_ref, bre_ref, bim_ref, cre_ref, cim_ref, sems,
            o_ref, osems,
            *sm_bufs):
    i = pl.program_id(0)
    s_bufs = sm_bufs[:2 * HB]
    m_bufs = sm_bufs[2 * HB:]

    def x_copy(b):
        return pltpu.make_async_copy(x_hbm.at[pl.ds(b * TQ, TQ)], x_ref.at[pl.ds(b * TQ, TQ)],
                                     sems.at[b])

    w_pairs = ((wq_hbm, wq_ref), (wkt_hbm, wkt_ref), (wvt_hbm, wvt_ref), (wo_hbm, wo_ref),
               (bre_hbm, bre_ref), (bim_hbm, bim_ref), (cre_hbm, cre_ref), (cim_hbm, cim_ref))

    def w_copy(n):
        return pltpu.make_async_copy(w_pairs[n][0], w_pairs[n][1], sems.at[NB + n])

    def o_copy(blk, t):
        return pltpu.make_async_copy(o_ref.at[pl.ds(t * RC, RC)],
                                     o_hbm.at[pl.ds(blk * TQ + t * RC, RC)], osems.at[t])

    def q_slice(h, blk):
        ro = pl.multiple_of(h * DH, DH)
        co = pl.multiple_of(blk * TQ, TQ)
        return qt_s[pl.ds(ro, DH), pl.ds(co, TQ)]

    def qk_chunk(c, qh):
        rows = slice(c * KC, (c + 1) * KC)
        return jnp.dot(k_s[rows, :], qh, preferred_element_type=F32)

    @pl.when(i == 0)
    def _init():
        x_copy(0).start()
        for n in (0, 1, 2):
            w_copy(n).start()
        for b in range(1, NB):
            x_copy(b).start()
        for n in range(3, N_W):
            w_copy(n).start()

        lre = lre_ref[...].astype(F32).reshape(1, P)
        lim = lim_ref[...].astype(F32).reshape(1, P)
        dt = jnp.exp(ldt_ref[...].astype(F32).reshape(1, P)).astype(BF16).astype(F32)
        zr = dt * lre
        zi = dt * lim
        er = jnp.exp(zr)
        l1r = er * jnp.cos(zi)
        l1i = er * jnp.sin(zi)
        nr = l1r - 1.0
        ni = l1i
        den = lre * lre + lim * lim
        c_r = (nr * lre + ni * lim) / den
        c_i = (ni * lre - nr * lim) / den
        pows = [(l1r, l1i)]
        for _ in range(7):
            pr, pi = pows[-1]
            pows.append(_cmul(pr, pi, l1r, l1i))

        rows = lax.broadcasted_iota(jnp.int32, (8, P), 0)

        def masked(v, k):
            return jnp.where(rows >= k, jnp.broadcast_to(v, (8, P)), 0.0)

        tab_s[0] = masked(pows[0][0], 1)
        tab_s[1] = masked(pows[0][1], 1)
        tab_s[2] = masked(pows[1][0], 2)
        tab_s[3] = masked(pows[1][1], 2)
        tab_s[4] = masked(pows[3][0], 4)
        tab_s[5] = masked(pows[3][1], 4)
        tr = jnp.zeros((8, P), F32)
        ti = jnp.zeros((8, P), F32)
        for r in range(8):
            tr = jnp.where(rows == r, jnp.broadcast_to(pows[r][0], (8, P)), tr)
            ti = jnp.where(rows == r, jnp.broadcast_to(pows[r][1], (8, P)), ti)
        tab_s[6] = tr
        tab_s[7] = ti
        tab_s[8] = jnp.broadcast_to(c_r, (8, P))
        tab_s[9] = jnp.broadcast_to(c_i, (8, P))
        car_s[...] = jnp.zeros_like(car_s)

        w_copy(0).wait()
        for b in range(NB):
            x_copy(b).wait()
            qt = lax.dot_general(wq_ref[...], x_ref[b * TQ:(b + 1) * TQ, :],
                                 (((0,), (1,)), ((), ())), preferred_element_type=F32)
            qt_s[:, b * TQ:(b + 1) * TQ] = (qt.astype(BF16).astype(F32) * 0.25).astype(BF16)

        w_copy(1).wait()
        w_copy(2).wait()
        wkvt = jnp.concatenate([wkt_ref[...], wvt_ref[...]], axis=0)
        kvt = lax.dot_general(wkvt, x_ref[...], (((1,), (1,)), ((), ())),
                              preferred_element_type=F32)
        k_s[...] = kvt[0:DH, :].T.astype(BF16)
        vt_s[...] = kvt[DH:2 * DH, :].astype(BF16)

        for hh in range(HB):
            qh = q_slice(hh, 0)
            macc = None
            for c in range(NC):
                sc = qk_chunk(c, qh)
                s_bufs[hh][c * KC:(c + 1) * KC, :] = sc
                mc = jnp.max(sc.reshape(KC // 8, 8, TQ), axis=0)
                macc = mc if macc is None else jnp.maximum(macc, mc)
            m_bufs[hh][...] = macc

    row0 = pl.multiple_of(i * TQ, TQ)

    def stage(h, s_cur, m_cur, s_nxt, m_nxt, do_qk=True):
        if do_qk:
            hn = h + HB
            wrap = hn // H
            hn = hn - wrap * H
            bn = jnp.minimum(i + wrap, NB - 1)
            qh = q_slice(hn, bn)
        m = jnp.max(m_cur[...], axis=0, keepdims=True)
        macc = None
        oacc = None
        lacc = None
        for c in range(NC):
            rows = slice(c * KC, (c + 1) * KC)
            if do_qk:
                sc = qk_chunk(c, qh)
                s_nxt[rows, :] = sc
                mc = jnp.max(sc.reshape(KC // 8, 8, TQ), axis=0)
                macc = mc if macc is None else jnp.maximum(macc, mc)
            e = jnp.exp(s_cur[rows, :] - m)
            oc = jnp.dot(vt_s[:, rows], e.astype(BF16), preferred_element_type=F32)
            oacc = oc if oacc is None else oacc + oc
            lc = jnp.sum(e.reshape(KC // 8, 8, TQ), axis=0)
            lacc = lc if lacc is None else lacc + lc
        if do_qk:
            m_nxt[...] = macc
        off = pl.multiple_of(h * DH, DH)
        den = jnp.sum(lacc, axis=0, keepdims=True)
        at_s[pl.ds(off, DH), :] = (oacc / den).astype(BF16)

    def step(j, carry):
        def even():
            for r in range(HB):
                stage(HB * j + r, s_bufs[r], m_bufs[r], s_bufs[HB + r], m_bufs[HB + r])

        def odd():
            for r in range(HB):
                stage(HB * j + r, s_bufs[HB + r], m_bufs[HB + r], s_bufs[r], m_bufs[r])

        def last():
            for r in range(HB):
                stage(HB * j + r, s_bufs[HB + r], m_bufs[HB + r], None, None, do_qk=False)

        is_last = jnp.logical_and(i == NB - 1, j == H // HB - 1)
        lax.cond(is_last, last, lambda: lax.cond(j % 2 == 0, even, odd))
        return carry

    lax.fori_loop(0, H // HB, step, 0)

    def bproj(t):
        xt = x_ref[pl.ds(row0 + t * RC, RC), :]
        ur = lax.dot_general(xt, bre_ref[...], (((1,), (1,)), ((), ())),
                             preferred_element_type=F32)
        ui = lax.dot_general(xt, bim_ref[...], (((1,), (1,)), ((), ())),
                             preferred_element_type=F32)
        return ur, ui

    def scan(ur, ui):
        c_r = tab_s[8][0:1, :]
        c_i = tab_s[9][0:1, :]
        br = c_r * ur - c_i * ui
        bi = c_r * ui + c_i * ur
        G = RC // 8
        xr = br.reshape(G, 8, P)
        xi = bi.reshape(G, 8, P)
        for lvl, k in enumerate((1, 2, 4)):
            mr = tab_s[2 * lvl][None]
            mi = tab_s[2 * lvl + 1][None]
            sr = pltpu.roll(xr, k, 1)
            si = pltpu.roll(xi, k, 1)
            xr, xi = xr + mr * sr - mi * si, xi + mr * si + mi * sr
        hr = car_s[0:1, :]
        hi = car_s[1:2, :]
        tr = tab_s[6]
        ti = tab_s[7]
        outs_r = []
        outs_i = []
        for g in range(G):
            hb_r = jnp.broadcast_to(hr, (8, P))
            hb_i = jnp.broadcast_to(hi, (8, P))
            fr = xr[g] + tr * hb_r - ti * hb_i
            fi = xi[g] + tr * hb_i + ti * hb_r
            outs_r.append(fr)
            outs_i.append(fi)
            hr = fr[7:8, :]
            hi = fi[7:8, :]
        car_s[0:1, :] = hr
        car_s[1:2, :] = hi
        return (jnp.concatenate(outs_r, axis=0).astype(BF16),
                jnp.concatenate(outs_i, axis=0).astype(BF16))

    def finish(t, h_r, h_i):
        cols = slice(t * RC, (t + 1) * RC)
        a = lax.dot_general(at_s[:, cols], wo_ref[...], (((0,), (0,)), ((), ())),
                            preferred_element_type=F32)
        a_bf = a.astype(BF16)
        yr = lax.dot_general(h_r, cre_ref[...], (((1,), (1,)), ((), ())),
                             preferred_element_type=F32)
        yi = lax.dot_general(h_i, cim_ref[...], (((1,), (1,)), ((), ())),
                             preferred_element_type=F32)
        xt32 = x_ref[pl.ds(row0 + t * RC, RC), :].astype(F32)
        dskip = dskip_ref[...].astype(F32).reshape(1, D)
        b = 2.0 * (yr - yi) + (xt32 * dskip).astype(BF16).astype(F32)
        gw = gw_ref[...].astype(F32).reshape(1, D)
        prod = (xt32 * gw).astype(BF16).astype(F32)
        logit = jnp.sum(prod, axis=-1, keepdims=True).astype(BF16).astype(F32)
        g = jax.nn.sigmoid(logit).astype(BF16)
        one_m_g = (1.0 - g.astype(F32)).astype(BF16).astype(F32)
        ga = (g.astype(F32) * a_bf.astype(F32)).astype(BF16).astype(F32)
        o_ref[cols, :] = ga + one_m_g * b
        o_copy(i, t).start()

    @pl.when(i == 0)
    def _wait_rest():
        for n in range(3, N_W):
            w_copy(n).wait()

    @pl.when(i > 0)
    def _wait_prev_out():
        prev = jnp.maximum(i - 1, 0)
        for t in range(NT):
            o_copy(prev, t).wait()

    u = bproj(0)
    for t in range(NT):
        u_next = bproj(t + 1) if t + 1 < NT else None
        h_r, h_i = scan(*u)
        finish(t, h_r, h_i)
        u = u_next

    @pl.when(i == NB - 1)
    def _wait_last_out():
        for t in range(NT):
            o_copy(i, t).wait()


@jax.jit
def pallas_gated_mix__grouped_kv_mqa__ssm_conv_s5__prompt_kernel(
    A_x, A_wq, A_wk, A_wv, A_wo, B_x, B_Lambda_re, B_Lambda_im, B_B_re, B_B_im,
    B_C_re, B_C_im, B_log_dt, B_Dskip, gate_w,
):
    x = A_x.reshape(S_LEN, D)
    full = lambda shp: pl.BlockSpec(shp, lambda i: (0,) * len(shp))
    hbm = pl.BlockSpec(memory_space=pl.ANY)
    out = pl.pallas_call(
        _kernel,
        grid=(NB,),
        in_specs=[
            hbm, hbm, hbm, hbm, hbm,
            full((P,)), full((P,)),
            hbm, hbm, hbm, hbm,
            full((P,)), full((D,)), full((D,)),
        ],
        out_specs=pl.BlockSpec(memory_space=pl.ANY),
        out_shape=jax.ShapeDtypeStruct((S_LEN, D), F32),
        scratch_shapes=[
            pltpu.VMEM((S_LEN, DH), BF16),
            pltpu.VMEM((DH, S_LEN), BF16),
            pltpu.VMEM((D, S_LEN), BF16),
            pltpu.VMEM((D, TQ), BF16),
            pltpu.VMEM((10, 8, P), F32),
            pltpu.VMEM((8, P), F32),
            pltpu.VMEM((S_LEN, D), BF16),
            pltpu.VMEM((D, H * DH), BF16),
            pltpu.VMEM((DH, D), BF16),
            pltpu.VMEM((DH, D), BF16),
            pltpu.VMEM((H * DH, D), BF16),
            pltpu.VMEM((P, D), BF16),
            pltpu.VMEM((P, D), BF16),
            pltpu.VMEM((D, P), BF16),
            pltpu.VMEM((D, P), BF16),
            pltpu.SemaphoreType.DMA((NB + N_W,)),
            pltpu.VMEM((TQ, D), F32),
            pltpu.SemaphoreType.DMA((NT,)),
        ] + [pltpu.VMEM((S_LEN, TQ), F32)] * (2 * HB) + [pltpu.VMEM((8, TQ), F32)] * (2 * HB),
        compiler_params=pltpu.CompilerParams(
            dimension_semantics=("arbitrary",),
            vmem_limit_bytes=110 * 1024 * 1024,
        ),
    )(x, A_wq, A_wk.T, A_wv.T, A_wo, B_Lambda_re, B_Lambda_im, B_B_re, B_B_im,
      B_C_re, B_C_im, B_log_dt, B_Dskip, gate_w)
    return out.reshape(1, S_LEN, D)
```
